```python
import jax
import jax.numpy as jnp

def _softmax(x, axis=-1):
    return jax.nn.softmax(x, axis=axis)
def _gelu(x):
    return jax.nn.gelu(x, approximate=True)
def _silu(x):
    return jax.nn.silu(x)
def _sigmoid(x):
    return jax.nn.sigmoid(x)
def _layernorm(x, axis=-1, eps=1e-5):
    m = jnp.mean(x, axis=axis, keepdims=True)
    v = jnp.var(x, axis=axis, keepdims=True)
    return (x - m) / jnp.sqrt(v + eps)
def _scatter_add(tgt, idx, src, axis=0):
    return tgt.at[idx].add(src)
def _segment_sum(src, seg, n):
    return jax.ops.segment_sum(src, seg, n)
class _Rng:
    def __init__(self, key):
        self._k = key
    def _next(self):
        self._k, sub = jax.random.split(self._k)
        return sub
    def normal(self, shape):
        return jax.random.normal(self._next(), shape, dtype=jnp.bfloat16)
    def randint(self, lo, hi, shape):
        return jax.random.randint(self._next(), shape, lo, hi, dtype=jnp.int32)
    def uniform(self, shape, lo=0.0, hi=1.0):
        return jax.random.uniform(self._next(), shape, jnp.bfloat16, lo, hi)
    def permutation(self, n):
        return jax.random.permutation(self._next(), n)


kernel_name = 'concat_heads__gqa_block_cached__mha_block_cached__near_ridge'

def setup_inputs():
    _rng = _Rng(jax.random.key(int.from_bytes(__import__("os").urandom(4), "little")))
    _w = (lambda a: (lambda t: t.astype(jnp.bfloat16) if jnp.issubdtype(t.dtype, jnp.floating) else t)(jnp.asarray(a)))
    def _A_setup():
        B, Sq, D = 16, 160, 640
        Hq, Hkv, Sk, Dh = 32, 32, 512, 192
        assert Hq % Hkv == 0, (Hq, Hkv)
        return {
            "x": _w((lambda *s: _rng.normal(s) * 0.05)(B, Sq, D)),
            "k_cache": _w((lambda *s: _rng.normal(s) * 0.05)(B, Hkv, Sk, Dh)),
            "v_cache": _w((lambda *s: _rng.normal(s) * 0.05)(B, Hkv, Sk, Dh)),
            "wq": _w((lambda *s: _rng.normal(s) * 0.05)(D, Hq * Dh) * (D ** -0.5)),
            "wo": _w((lambda *s: _rng.normal(s) * 0.05)(Hq * Dh, D) * ((Hq * Dh) ** -0.5)),
        }
    _A_in = _A_setup()

    def _B_setup():
        B, Sq, D = 16, 160, 640
        H, Sk, Dh = 32, 512, 192
        return {
            "x": _w((lambda *s: _rng.normal(s) * 0.05)(B, Sq, D)),
            "k_cache": _w((lambda *s: _rng.normal(s) * 0.05)(B, H, Sk, Dh)),
            "v_cache": _w((lambda *s: _rng.normal(s) * 0.05)(B, H, Sk, Dh)),
            "wq": _w((lambda *s: _rng.normal(s) * 0.05)(D, H * Dh) * (D ** -0.5)),
            "wo": _w((lambda *s: _rng.normal(s) * 0.05)(H * Dh, D) * ((H * Dh) ** -0.5)),
        }
    _B_in = _B_setup()

    return {
        "A_x": _A_in["x"],
        "A_k_cache": _A_in["k_cache"],
        "A_v_cache": _A_in["v_cache"],
        "A_wq": _A_in["wq"],
        "A_wo": _A_in["wo"],
        "B_x": _B_in["x"],
        "B_k_cache": _B_in["k_cache"],
        "B_v_cache": _B_in["v_cache"],
        "B_wq": _B_in["wq"],
        "B_wo": _B_in["wo"],
    }

def reference(A_x, A_k_cache, A_v_cache, A_wq, A_wo, B_x, B_k_cache, B_v_cache, B_wq, B_wo):
    def _A_ref(x, k_cache, v_cache, wq, wo):
        B, Sq, D = x.shape
        Hq, Dh = 32, 192
        Hkv = k_cache.shape[1]
        rep = Hq // Hkv
        q = (lambda x, *d: x.transpose(*d))((x @ wq).reshape(B, Sq, Hq, Dh), 0, 2, 1, 3)
        k = jnp.repeat(k_cache, rep, axis=1)
        v = jnp.repeat(v_cache, rep, axis=1)
        scores = jnp.einsum("bhqd,bhkd->bhqk", q, k) * (Dh ** -0.5)
        p = _softmax(scores, axis=-1)
        o = jnp.einsum("bhqk,bhkd->bhqd", p, v)
        return (lambda x, *d: x.transpose(*d))(o, 0, 2, 1, 3).reshape(B, Sq, Hq * Dh) @ wo

    def _B_ref(x, k_cache, v_cache, wq, wo):
        B, Sq, D = x.shape
        H, Dh = 32, 192
        q = (lambda x, *d: x.transpose(*d))((x @ wq).reshape(B, Sq, H, Dh), 0, 2, 1, 3)
        scores = jnp.einsum("bhqd,bhkd->bhqk", q, k_cache) * (Dh ** -0.5)
        p = _softmax(scores, axis=-1)
        o = jnp.einsum("bhqk,bhkd->bhqd", p, v_cache)
        return (lambda x, *d: x.transpose(*d))(o, 0, 2, 1, 3).reshape(B, Sq, H * Dh) @ wo

    a = _A_ref(A_x, A_k_cache, A_v_cache, A_wq, A_wo)
    b = _B_ref(B_x, B_k_cache, B_v_cache, B_wq, B_wo)
    return jnp.concatenate([a, b], axis=-1)
```

```python
import functools

import jax
import jax.experimental.pallas as pl
import jax.experimental.pallas.tpu as pltpu
import jax.numpy as jnp
import numpy as np

B, SQ, D = 16, 160, 640
H, SK, DH = 32, 512, 192

LANES = 128
HALF = LANES // 2
PAIR = 2 * DH
HS = SQ // 2
Q_SCALE = float(DH ** -0.5 * np.log2(np.e))

NBAT, NPAIR = 4, 2
STEP = 2
LEAD = 8
NSLOT = 6

NBB = B // NBAT
NGQ = H // (2 * NPAIR)
WIDTH = NPAIR * PAIR
NGROUP = 2 * NGQ
NUNIT = NGROUP * NBB
AHEAD = NSLOT - STEP
LEAD_GROUPS = LEAD // NBB
assert LEAD % NBB == 0 and NBB % STEP == 0 and 2 * AHEAD <= LEAD <= NUNIT // 2 - NBB

F32, BF16 = jnp.float32, jnp.bfloat16


def _mm(a, b):
    return jnp.dot(a, b, preferred_element_type=F32)


def _mm_nt(a, b):
    return jax.lax.dot_general(a, b, (((1,), (1,)), ((), ())), preferred_element_type=F32)


def _bf16(a):
    return a.astype(BF16)


def _round(a):
    return a.astype(BF16).astype(F32)


def _low_lanes(rows):
    return jax.lax.broadcasted_iota(jnp.int32, (rows, LANES), 1) < HALF


def _softmax_parts(s):
    p = _bf16(jnp.exp2(s - jnp.max(s, axis=1, keepdims=True)))
    total = jnp.sum(p.astype(F32), axis=1, keepdims=True)
    r = pl.reciprocal(total, approx=True)
    return p, r * (2.0 - total * r)


class _HeadPair:
    def __init__(self, x_ref, wq_ref, kt_ref, vt_ref, wo_ref, acc_ref):
        self.x_ref, self.wq_ref = x_ref, wq_ref
        self.kt_ref, self.vt_ref = kt_ref, vt_ref
        self.wo_ref, self.acc_ref = wo_ref, acc_ref
        self.p, self.r = [None, None], [None, None]

    def project_q(self):
        q = _mm(self.x_ref[...], self.wq_ref[...]) * Q_SCALE
        x0, x1, x2 = (q[:HS, t * LANES:(t + 1) * LANES] for t in range(3))
        y0, y1, y2 = (q[HS:, t * LANES:(t + 1) * LANES] for t in range(3))
        low = _low_lanes(HS)
        y_fa = pltpu.roll(jnp.where(low, y0, y2), HALF, 1)
        d_cd = y1 - _round(x1)
        lhs = [_bf16(a) for a in (
            x0 - jnp.where(low, 0.0, _round(y0)),
            jnp.where(low, d_cd, y_fa),
            jnp.where(low, x1, y0),
            x2 - jnp.where(low, _round(y2), 0.0),
            jnp.where(low, y_fa, d_cd),
            jnp.where(low, y2, x1),
        )]
        self.lhs = lambda i: lhs[i]
        return lhs

    def scores(self, h):
        parts = (((0, 1), (2, 0), (2, 1)), ((4, 5), (5, 3), (4, 3)))[h]
        k1, k2, k3 = (
            jnp.concatenate([self.kt_ref[i * HALF:(i + 1) * HALF, :] for i in ij], axis=0)
            for ij in parts)
        shared = _mm(self.lhs(3 * h + 2), k3)
        px, rx = _softmax_parts(_mm(self.lhs(3 * h), k1) + shared)
        py, ry = _softmax_parts(_mm(self.lhs(3 * h + 1), k2) + shared)
        self.p[h] = jnp.concatenate([px, py], axis=0)
        self.r[h] = jnp.concatenate([rx, ry], axis=0)

    def values_0(self):
        p, vt = self.p[0], self.vt_ref
        ot = _mm_nt(vt[0:DH, :], p[:LANES])
        rest = _mm_nt(p[LANES:], vt[0:LANES, :])
        self.o_ab = _bf16(jnp.concatenate([ot[:LANES].T, rest], axis=0) * self.r[0])
        self.ot_c = ot[LANES:]

    def values_1(self):
        p, vt = self.p[1], self.vt_ref
        ot = _mm_nt(vt[DH:PAIR, :], p[:LANES])
        rest_ef = _mm_nt(p[LANES:], vt[2 * LANES:PAIR, :])
        both = _mm_nt(jnp.concatenate([self.p[0][LANES:], p[LANES:]], axis=0),
                      vt[LANES:2 * LANES, :])
        n = SQ - LANES
        o_cd = jnp.concatenate(
            [jnp.concatenate([self.ot_c, ot[:HALF]], axis=0).T,
             jnp.where(_low_lanes(n), both[:n], both[n:])], axis=0)
        o_cd = _bf16(o_cd * jnp.where(_low_lanes(SQ), self.r[0], self.r[1]))
        o_ef = _bf16(jnp.concatenate([ot[HALF:].T, rest_ef], axis=0) * self.r[1])
        self.o = jnp.concatenate([self.o_ab, o_cd, o_ef], axis=1)

    def project_o(self):
        self.acc_ref[...] += _mm(self.o, self.wo_ref[...])


def _run_stages(pairs, with_q):
    n = len(pairs)
    for t in range(-1, n + 2):
        if with_q and t + 1 < n:
            pairs[t + 1].project_q()
        if 0 <= t < n:
            pairs[t].scores(0)
            pairs[t].scores(1)
        if 0 <= t - 1 < n:
            pairs[t - 1].values_0()
            pairs[t - 1].values_1()
        if 0 <= t - 2 < n:
            pairs[t - 2].project_o()


def _kernel(ax, ak, av, awq, awo, bx, bk, bv, bwq, bwo, out,
            x_buf, q_buf, k_buf, v_buf, wq_buf, wo_buf, acc, out_buf,
            x_sem, kv_sem, wq_sem, wo_sem, out_sem):
    xs, ks, vs, wqs, wos = (ax, bx), (ak, bk), (av, bv), (awq, bwq), (awo, bwo)

    def columns(g):
        return pl.ds(pl.multiple_of((g % NGQ) * WIDTH, WIDTH), WIDTH)

    def batches(bb):
        return pl.ds(bb * NBAT, NBAT)

    def x_copies(br, i):
        return [pltpu.make_async_copy(xs[br].at[batches(i)], x_buf.at[br, batches(i)], x_sem.at[br, i])]

    def kv_copies(br, i):
        return [pltpu.make_async_copy(src[br].at[batches(i % NBB), columns(i // NBB), :],
                                      buf.at[i % NSLOT], kv_sem.at[i % NSLOT, j])
                for j, (src, buf) in enumerate(((ks, k_buf), (vs, v_buf)))]

    def wq_copies(br, i):
        return [pltpu.make_async_copy(wqs[br].at[:, columns(i)], wq_buf.at[i], wq_sem.at[i])]

    def wo_copies(br, i):
        return [pltpu.make_async_copy(wos[br].at[columns(i), :], wo_buf.at[i], wo_sem.at[i])]

    def out_copies(br, i):
        return [pltpu.make_async_copy(out_buf.at[br, batches(i % NBB)],
                                      out.at[batches(i % NBB), :, pl.ds(br * D, D)], out_sem.at[br, i % NBB])]

    def start(copies):
        for copy in copies:
            copy.start()

    def wait(copies):
        for copy in copies:
            copy.wait()

    def start_any(copies, i, per_branch, cond=True):
        for br in range(2):
            @pl.when(cond & (i >= br * per_branch) & (i < (br + 1) * per_branch))
            def _():
                start(copies(br, i))

    def head_pairs(u):
        g, bb, slot = u // NBB, u % NBB, u % NSLOT
        br = g // NGQ
        return [_HeadPair(x_buf.at[br, bb * NBAT + j],
                          wq_buf.at[g, :, pl.ds(p * PAIR, PAIR)],
                          k_buf.at[slot, j, pl.ds(p * PAIR, PAIR)],
                          v_buf.at[slot, j, pl.ds(p * PAIR, PAIR)],
                          wo_buf.at[g, pl.ds(p * PAIR, PAIR)],
                          acc.at[br, bb * NBAT + j])
                for j in range(NBAT) for p in range(NPAIR)]

    def lead_q(u, carry):
        @pl.when(u % NBB == 0)
        def _():
            wait(wq_copies(0, u // NBB))

        @pl.when(u < NBB)
        def _():
            wait(x_copies(0, u))

        @pl.when(u == 0)
        def _():
            for i in range(1, NBB):
                start(x_copies(0, i))
            for i in range(1, LEAD_GROUPS):
                start(wq_copies(0, i))
            start(wo_copies(0, 0))

        @pl.when((u % 2 == 1) & (u // 2 < AHEAD))
        def _():
            start(kv_copies(0, u // 2))

        for i, pair in enumerate(head_pairs(u)):
            for j, lhs in enumerate(pair.project_q()):
                q_buf[u, i, j] = lhs
        return carry

    def attend(it, carry, with_q):
        n = STEP if with_q else 1
        u = it * n
        g, bb = u // NBB, u % NBB

        @pl.when(bb == 0)
        def _():
            wait(wo_copies(0, g))
            if with_q:
                wait(wq_copies(0, g))

        if with_q:
            @pl.when(u == NUNIT // 2)
            def _():
                for i in range(NBB):
                    wait(x_copies(1, i))

        for d in range(n):
            wait(kv_copies(0, u + d))

        start_any(wq_copies, g + 1, NGQ, (bb == 0) & (g + 1 >= LEAD_GROUPS))
        start_any(wo_copies, g + 1, NGQ, bb == 0)
        if with_q:
            @pl.when(u == NUNIT // 2 - NBB)
            def _():
                for i in range(NBB):
                    start(x_copies(1, i))

        for d in range(n):
            start_any(kv_copies, u + AHEAD + d, NUNIT // 2)

        pairs = [pair for d in range(n) for pair in head_pairs(u + d)]
        if not with_q:
            for i, pair in enumerate(pairs):
                pair.lhs = functools.partial(lambda i, j: q_buf[u, i, j], i)
        _run_stages(pairs, with_q)

        if with_q:
            @pl.when(g % NGQ == NGQ - 1)
            def _():
                for d in range(n):
                    out_buf[g // NGQ, batches(bb + d)] = _bf16(acc[g // NGQ, batches(bb + d)])
                    start_any(out_copies, u + d, NUNIT // 2)
        return carry

    start(wq_copies(0, 0) + x_copies(0, 0))
    acc[...] = jnp.zeros(acc.shape, F32)
    jax.lax.fori_loop(0, LEAD, lead_q, 0)
    jax.lax.fori_loop(0, LEAD, functools.partial(attend, with_q=False), 0)
    jax.lax.fori_loop(LEAD // STEP, NUNIT // STEP, functools.partial(attend, with_q=True), 0)
    for br in range(2):
        for i in range(NBB):
            wait(out_copies(br, i))


@jax.jit
def pallas_concat_heads__gqa_block_cached__mha_block_cached__near_ridge_kernel(
    A_x: jax.Array,
    A_k_cache: jax.Array,
    A_v_cache: jax.Array,
    A_wq: jax.Array,
    A_wo: jax.Array,
    B_x: jax.Array,
    B_k_cache: jax.Array,
    B_v_cache: jax.Array,
    B_wq: jax.Array,
    B_wo: jax.Array,
):
    def transposed(cache):
        assert cache.shape == (B, H, SK, DH), cache.shape
        return jnp.swapaxes(cache, 2, 3).reshape(B, H * DH, SK)

    hbm = pl.BlockSpec(memory_space=pl.ANY)
    dma = pltpu.SemaphoreType.DMA
    return pl.pallas_call(
        _kernel,
        in_specs=[hbm] * 10,
        out_specs=hbm,
        out_shape=jax.ShapeDtypeStruct((B, SQ, 2 * D), BF16),
        scratch_shapes=[
            pltpu.VMEM((2, B, SQ, D), BF16),
            pltpu.VMEM((LEAD, NBAT * NPAIR, 6, HS, LANES), BF16),
            pltpu.VMEM((NSLOT, NBAT, WIDTH, SK), BF16),
            pltpu.VMEM((NSLOT, NBAT, WIDTH, SK), BF16),
            pltpu.VMEM((NGROUP, D, WIDTH), BF16),
            pltpu.VMEM((NGROUP, WIDTH, D), BF16),
            pltpu.VMEM((2, B, SQ, D), F32),
            pltpu.VMEM((2, B, SQ, D), BF16),
            dma((2, NBB)), dma((NSLOT, 2)), dma((NGROUP,)), dma((NGROUP,)), dma((2, NBB)),
        ],
        compiler_params=pltpu.CompilerParams(
            vmem_limit_bytes=124 * 1024 * 1024, disable_bounds_checks=True),
        name="attn_kernel",
    )(A_x, transposed(A_k_cache), transposed(A_v_cache), A_wq, A_wo,
      B_x, transposed(B_k_cache), transposed(B_v_cache), B_wq, B_wo)
```

```python
import functools

import jax
import jax.experimental.pallas as pl
import jax.experimental.pallas.tpu as pltpu
import jax.numpy as jnp
import numpy as np

B, SQ, D = 16, 160, 640
H, SK, DH = 32, 512, 192

LANES = 128
HALF = LANES // 2
PAIR = 2 * DH
HS = SQ // 2
REST = (SQ - LANES) // 2
Q_SCALE = float(DH ** -0.5 * np.log2(np.e))

NBAT, NPAIR = 4, 2
STEP = 2
LEAD = 8
NSLOT = 6
FIRST = 2

NBB = B // NBAT
NGQ = H // (2 * NPAIR)
WIDTH = NPAIR * PAIR
NGROUP = 2 * NGQ
NUNIT = NGROUP * NBB
AHEAD = NSLOT - STEP
LEAD_GROUPS = LEAD // NBB
assert NPAIR == 2 and LEAD == 2 * NBB and NBB % STEP == 0
assert 2 * AHEAD <= LEAD <= NUNIT // 2 - NBB

PARTS = (((0, 1), (2, 0), (2, 1)), ((4, 5), (5, 3), (4, 3)))

SCHEDULE = "p p p p K00 S01 K02 K10 K12 K01 K11 S10 V0 S02 P P S00 V1 S12 S11 p F p"
SCHEDULE_LEAD = "K00 K02 S00 K10 K12 S10 V0 S02 P P K01 K11 S12 V1 S01 S11 F P"
Q_LEAD, O_LAG = 2, 3

F32, BF16 = jnp.float32, jnp.bfloat16


def _mm(a, b):
    return jnp.dot(a, b, preferred_element_type=F32)


def _mm_nt(a, b):
    return jax.lax.dot_general(a, b, (((1,), (1,)), ((), ())), preferred_element_type=F32)


def _bf16(a):
    return a.astype(BF16)


def _round(a):
    return a.astype(BF16).astype(F32)


def _tile(i):
    return slice(i * LANES, (i + 1) * LANES)


def _low_lanes(rows):
    return jax.lax.broadcasted_iota(jnp.int32, (rows, LANES), 1) < HALF


def _inverse_row_sum(p):
    total = jnp.sum(p, axis=1, keepdims=True)
    r = pl.reciprocal(total, approx=True)
    return r * (2.0 - total * r)


def _div(a, n):
    return a >> (n.bit_length() - 1)


def _mod(a, n):
    return a & (n - 1)


class _HeadPair:
    def __init__(self, x_ref, wq_ref, kt_ref, vt_ref, wo_ref, acc_ref):
        self.x_ref, self.wq_ref = x_ref, wq_ref
        self.kt_ref, self.vt_ref = kt_ref, vt_ref
        self.wo_ref, self.acc_ref = wo_ref, acc_ref
        self.out_ref = self.on_done = None
        self.shared, self.p, self.r, self.p_rest = {}, {}, {}, {}
        self.ot, self.o_rest = {}, {}

    def q_tiles(self):
        q = [None] * 3

        def tile(n, k):
            part = _mm(self.x_ref[:, _tile(k)], self.wq_ref[_tile(k), _tile(n)])
            q[n] = part if k == 0 else q[n] + part
            if (n, k) == (2, D // LANES - 1):
                self._make_lhs([a * Q_SCALE for a in q])

        return [functools.partial(tile, n, k) for n in range(3) for k in range(D // LANES)]

    def _make_lhs(self, q):
        low = _low_lanes(HS)
        x0, x1, x2 = (a[:HS] for a in q)
        y0, y1, y2 = (a[HS:] for a in q)
        y_50 = pltpu.roll(jnp.where(low, y0, y2), HALF, 1)
        d_23 = y1 - _round(x1)
        self.lhs = [_bf16(a) for a in (
            x0 - jnp.where(low, 0.0, _round(y0)),
            jnp.where(low, d_23, y_50),
            jnp.where(low, x1, y0),
            x2 - jnp.where(low, _round(y2), 0.0),
            jnp.where(low, y_50, d_23),
            jnp.where(low, y2, x1),
        )]

    @staticmethod
    def _weights(ref, h, i):
        return jnp.concatenate([ref[j * HALF:(j + 1) * HALF, :] for j in PARTS[h][i]], axis=0)

    def K(self, h, i):
        if i == 0:
            self.shared[h] = _mm(self.lhs[3 * h + 2], self._weights(self.kt_ref, h, 2))
            return
        s = _mm(self.lhs[3 * h + i - 1], self._weights(self.kt_ref, h, i - 1)) + self.shared[h]
        e = jnp.exp2(s - jnp.max(s, axis=1, keepdims=True))
        if i == 2:
            rest = e[LANES - HS:]
            rest = rest * _inverse_row_sum(rest)
            x, y = rest[:REST], rest[REST:]
            self.p_rest[h] = (_bf16(x), _bf16(y), _bf16(x + y))
            e = e[:LANES - HS]
        self.p[h, i] = _bf16(e)
        self.r[h, i] = _inverse_row_sum(self.p[h, i].astype(F32))

    def V(self, h):
        p = jnp.concatenate([self.p[h, 1], self.p[h, 2]], axis=0)
        self.ot[h] = _mm_nt(self.vt_ref[h * DH:(h + 1) * DH, :], p)

    def S(self, h, i):
        self.o_rest[h, i] = _mm_nt(self.p_rest[h][i], self._weights(self.vt_ref, h, i))

    def F(self):
        r0, r1 = (jnp.concatenate([self.r[h, 1], self.r[h, 2]], axis=0) for h in range(2))
        ot0, ot1 = self.ot[0], self.ot[1]
        top = (ot0[:LANES].T, jnp.concatenate([ot0[LANES:], ot1[:HALF]], axis=0).T, ot1[HALF:].T)
        low = _low_lanes(REST)
        a1, a2, a3 = (self.o_rest[0, i] for i in range(3))
        b1, b2, b3 = (self.o_rest[1, i] for i in range(3))
        y_05 = pltpu.roll(jnp.where(low, b2, a2), HALF, 1)
        ox = (a1, jnp.where(low, a3 - a2, b3 - b2), b1)
        oy = (jnp.where(low, y_05, a3 - a1), jnp.where(low, a2, b2), jnp.where(low, b3 - b1, y_05))
        scale = (r0, jnp.where(_low_lanes(LANES), r0, r1), r1)
        self.o = [jnp.concatenate([_bf16(t * r), _bf16(x), _bf16(y)], axis=0)
                  for t, r, x, y in zip(top, scale, ox, oy)]

    def o_tiles(self):
        total = [None]

        def tile(n, k):
            part = _mm(self.o[k], self.wo_ref[_tile(k), _tile(n)])
            total[0] = part if k == 0 else total[0] + part
            if k == 2:
                new = self.acc_ref[:, _tile(n)] + total[0]
                self.acc_ref[:, _tile(n)] = new
                if self.out_ref is not None:
                    self.out_ref[:, _tile(n)] = _bf16(new)
                    if n == D // LANES - 1:
                        self.on_done()

        return [functools.partial(tile, n, k) for n in range(D // LANES) for k in range(3)]


def _run_schedule(schedule, pairs, with_q):
    queue = []

    def issue(count):
        for tile in queue[:count]:
            tile()
        del queue[:count]

    n = len(pairs)
    for t in range(-Q_LEAD, n + O_LAG):
        if with_q and t + Q_LEAD < n:
            queue += pairs[t + Q_LEAD].q_tiles()
        if 0 <= t - O_LAG < n:
            queue += pairs[t - O_LAG].o_tiles()
        both = len(queue) >= 2 * 3 * (D // LANES)
        for op in schedule.split():
            if op in "Pp":
                if len(queue) >= 4 and (op == "P" or both):
                    issue(4)
                continue
            i = t if op[0] == "K" else t - 1
            if 0 <= i < n:
                pair = pairs[i]
                {"K": pair.K, "V": pair.V, "S": pair.S, "F": pair.F}[op[0]](*map(int, op[1:]))
        issue(len(queue) // 4 * 4)
    issue(len(queue))


class _Loads:
    def __init__(self, ref):
        self.ref = ref

    def __getitem__(self, i):
        return self.ref[i]


def _kernel(ax, ak, av, awq, awo, bx, bk, bv, bwq, bwo, out,
            x_buf, q_buf, k_buf, v_buf, wq_buf, wo_buf, acc, out_buf,
            x_sem, kv_sem, wq_sem, wo_sem, first_sem, out_sem):
    ks, vs, wqs, wos = (ak, bk), (av, bv), (awq, bwq), (awo, bwo)

    def columns(g):
        return pl.ds(pl.multiple_of(_mod(g, NGQ) * WIDTH, WIDTH), WIDTH)

    def batches(bb):
        return pl.ds(bb * NBAT, NBAT)

    def later_slot(slot, d):
        return jnp.where(slot + d >= NSLOT, slot + d - NSLOT, slot + d)

    def ax_copy(first, count, sem):
        rows = pl.ds(first, count)
        return pltpu.make_async_copy(ax.at[rows], x_buf.at[0, rows], x_sem.at[sem])

    ax_copies = [ax_copy(0, FIRST, 0), ax_copy(FIRST, NBAT - FIRST, 1)]
    ax_copies += [ax_copy(i * NBAT, NBAT, i + 1) for i in range(1, NBB)]
    bx_copy = pltpu.make_async_copy(bx, x_buf.at[1], x_sem.at[NBB + 1])

    def kv_copies(slot, br, i):
        return [pltpu.make_async_copy(src[br].at[batches(_mod(i, NBB)), columns(_div(i, NBB)), :],
                                      buf.at[slot], kv_sem.at[slot, j])
                for j, (src, buf) in enumerate(((ks, k_buf), (vs, v_buf)))]

    def wq_copies(br, i):
        return [pltpu.make_async_copy(wqs[br].at[:, columns(i)], wq_buf.at[i], wq_sem.at[_mod(i, 2)])]

    def wo_copies(br, i):
        return [pltpu.make_async_copy(wos[br].at[columns(i), :], wo_buf.at[i], wo_sem.at[_mod(i, 2)])]

    def out_copy(br, b):
        cols = pl.ds(pl.multiple_of(br * D, LANES), D)
        return pltpu.make_async_copy(out_buf.at[br, b], out.at[b, :, cols], out_sem)

    def start(copies):
        for copy in copies:
            copy.start()

    def wait(copies):
        for copy in copies:
            copy.wait()

    def on_branch(action, copies, i, per_branch, cond):
        for br in range(2):
            @pl.when(cond & (i >= br * per_branch) & (i < (br + 1) * per_branch))
            def _():
                action(copies(br, i))

    def head_pairs(u, slot):
        g, bb = _div(u, NBB), _mod(u, NBB)
        br = _div(g, NGQ)
        return [_HeadPair(x_buf.at[br, bb * NBAT + j],
                          wq_buf.at[g, :, pl.ds(p * PAIR, PAIR)],
                          k_buf.at[slot, j, pl.ds(p * PAIR, PAIR)],
                          v_buf.at[slot, j, pl.ds(p * PAIR, PAIR)],
                          wo_buf.at[g, pl.ds(p * PAIR, PAIR)],
                          acc.at[br, bb * NBAT + j])
                for j in range(NBAT) for p in range(NPAIR)]

    def project_lead(u, wanted):
        for i, pair in enumerate(head_pairs(u, 0)):
            if wanted(i):
                for tile in pair.q_tiles():
                    tile()
                for j, lhs in enumerate(pair.lhs):
                    q_buf[u, i, j] = lhs

    def clear_acc(u):
        acc[_div(u, NBB), batches(_mod(u, NBB))] = jnp.zeros((NBAT, SQ, D), F32)

    def lead(u, carry):
        @pl.when(_mod(u, NBB) == 0)
        def _():
            wait(wq_copies(0, _div(u, NBB)))

        for i in range(1, NBB):
            pl.when(u == i)(ax_copies[i + 1].wait)

        @pl.when((_mod(u, 2) == 1) & (_div(u, 2) < AHEAD))
        def _():
            start(kv_copies(_div(u, 2), 0, _div(u, 2)))

        clear_acc(u)
        project_lead(u, lambda i: True)
        return carry

    def attend(it, slot, with_q):
        n = STEP if with_q else 1
        u = it * n
        g, bb = _div(u, NBB), _mod(u, NBB)
        br = _div(g, NGQ)
        slots = [slot] + [later_slot(slot, d) for d in range(1, n)]

        @pl.when(bb == 0)
        def _():
            wait(wo_copies(0, g))
            if with_q:
                wait(wq_copies(0, g))

        if with_q:
            pl.when(u == NUNIT // 2)(bx_copy.wait)
        for d in range(n):
            wait(kv_copies(slots[d], 0, u + d))

        on_branch(start, wq_copies, g + 1, NGQ, (bb == 0) & (g + 1 >= LEAD_GROUPS))
        on_branch(start, wo_copies, g + 1, NGQ, bb == 0)
        if with_q:
            pl.when(u == NUNIT // 2 - NBB)(bx_copy.start)
        for d in range(n):
            on_branch(start, functools.partial(kv_copies, later_slot(slot, AHEAD + d)),
                      u + AHEAD + d, NUNIT // 2, True)

        def send(b):
            @pl.when(_mod(g, NGQ) == NGQ - 1)
            def _():
                out_copy(br, b).start()

        pairs = [pair for d in range(n) for pair in head_pairs(u + d, slots[d])]
        for i, pair in enumerate(pairs):
            if not with_q:
                pair.lhs = _Loads(q_buf.at[u, i])
            elif i % NPAIR == NPAIR - 1:
                b = bb * NBAT + i // NPAIR
                pair.out_ref, pair.on_done = out_buf.at[br, b], functools.partial(send, b)
        _run_schedule(SCHEDULE if with_q else SCHEDULE_LEAD, pairs, with_q)
        return later_slot(slot, n)

    first_wq = [pltpu.make_async_copy(awq.at[:, pl.ds(p * PAIR, PAIR)],
                                      wq_buf.at[0, :, pl.ds(p * PAIR, PAIR)], first_sem.at[p])
                for p in range(NPAIR)]

    def in_first_block(i):
        return i % NPAIR == 0 and i // NPAIR < FIRST

    start([first_wq[0], ax_copies[0], first_wq[1], ax_copies[1]])
    clear_acc(0)
    wait([first_wq[0], ax_copies[0]])
    project_lead(0, in_first_block)
    wait([first_wq[1], ax_copies[1]])
    start(ax_copies[2:])
    for g in range(1, LEAD_GROUPS):
        start(wq_copies(0, g))
    start(wo_copies(0, 0))
    project_lead(0, lambda i: not in_first_block(i))

    jax.lax.fori_loop(1, LEAD, lead, 0)
    slot = jax.lax.fori_loop(0, LEAD, functools.partial(attend, with_q=False), 0)
    jax.lax.fori_loop(LEAD // STEP, NUNIT // STEP, functools.partial(attend, with_q=True), slot)
    wait([out_copy(br, b) for br in range(2) for b in range(B)])


@jax.jit
def pallas_concat_heads__gqa_block_cached__mha_block_cached__near_ridge_kernel(
    A_x: jax.Array,
    A_k_cache: jax.Array,
    A_v_cache: jax.Array,
    A_wq: jax.Array,
    A_wo: jax.Array,
    B_x: jax.Array,
    B_k_cache: jax.Array,
    B_v_cache: jax.Array,
    B_wq: jax.Array,
    B_wo: jax.Array,
):
    def transposed(cache):
        assert cache.shape == (B, H, SK, DH), cache.shape
        return jnp.swapaxes(cache, 2, 3).reshape(B, H * DH, SK)

    hbm = pl.BlockSpec(memory_space=pl.ANY)
    dma = pltpu.SemaphoreType.DMA
    return pl.pallas_call(
        _kernel,
        in_specs=[hbm] * 10,
        out_specs=hbm,
        out_shape=jax.ShapeDtypeStruct((B, SQ, 2 * D), BF16),
        scratch_shapes=[
            pltpu.VMEM((2, B, SQ, D), BF16),
            pltpu.VMEM((LEAD, NBAT * NPAIR, 6, HS, LANES), BF16),
            pltpu.VMEM((NSLOT, NBAT, WIDTH, SK), BF16),
            pltpu.VMEM((NSLOT, NBAT, WIDTH, SK), BF16),
            pltpu.VMEM((NGROUP, D, WIDTH), BF16),
            pltpu.VMEM((NGROUP, WIDTH, D), BF16),
            pltpu.VMEM((2, B, SQ, D), F32),
            pltpu.VMEM((2, B, SQ, D), BF16),
            dma((NBB + 2,)), dma((NSLOT, 2)), dma((2,)), dma((2,)), dma((NPAIR,)), dma(()),
        ],
        compiler_params=pltpu.CompilerParams(
            vmem_limit_bytes=124 * 1024 * 1024, disable_bounds_checks=True),
        name="attn_kernel",
    )(A_x, transposed(A_k_cache), transposed(A_v_cache), A_wq, A_wo,
      B_x, transposed(B_k_cache), transposed(B_v_cache), B_wq, B_wo)
```

```python
import functools

import jax
import jax.experimental.pallas as pl
import jax.experimental.pallas.tpu as pltpu
import jax.numpy as jnp
import numpy as np

B, SQ, D = 16, 160, 640
H, SK, DH = 32, 512, 192

LANES = 128
HALF = LANES // 2
PAIR = 2 * DH
HS = SQ // 2
REST = (SQ - LANES) // 2
Q_SCALE = float(DH ** -0.5 * np.log2(np.e))

NBAT, NPAIR = 4, 2
STEP = 2
LEAD = 8
NSLOT = 6
FIRST = 2

NBB = B // NBAT
NGQ = H // (2 * NPAIR)
WIDTH = NPAIR * PAIR
NGROUP = 2 * NGQ
NUNIT = NGROUP * NBB
AHEAD = NSLOT - STEP
LEAD_GROUPS = LEAD // NBB
assert NPAIR == 2 and LEAD == 2 * NBB and NBB % STEP == 0
assert 2 * AHEAD <= LEAD <= NUNIT // 2 - NBB

PARTS = (((0, 1), (2, 0), (2, 1)), ((4, 5), (5, 3), (4, 3)))

SCHEDULE = (
    "K00 K10 S01 K02 K12 K01 S10 K11 V0 S02 P P S00 V1 S12 S11 F",
    "P P P K00 S01 K02 K10 P K12 K01 S10 V0 S02 P P S00 V1 S11 S12 P F P K11",
    "K00 S00 K10 K12 S10 V0 K02 S02 P P K01 K11 S12 V1 S01 S11 F P",
)
SCHEDULE_LEAD = ("K00 K02 S00 K10 K12 S10 V0 S02 P P K01 K11 S12 V1 S01 S11 F P",) * 3
Q_LEAD, O_LAG = 2, 3

F32, BF16 = jnp.float32, jnp.bfloat16


def _mm(a, b):
    return jnp.dot(a, b, preferred_element_type=F32)


def _mm_nt(a, b):
    return jax.lax.dot_general(a, b, (((1,), (1,)), ((), ())), preferred_element_type=F32)


def _bf16(a):
    return a.astype(BF16)


def _round(a):
    return a.astype(BF16).astype(F32)


def _tile(i):
    return slice(i * LANES, (i + 1) * LANES)


def _low_lanes(rows):
    return jax.lax.broadcasted_iota(jnp.int32, (rows, LANES), 1) < HALF


def _inverse_row_sum(p):
    total = jnp.sum(p, axis=1, keepdims=True)
    r = pl.reciprocal(total, approx=True)
    return r * (2.0 - total * r)


def _div(a, n):
    return a >> (n.bit_length() - 1)


def _mod(a, n):
    return a & (n - 1)


class _HeadPair:
    def __init__(self, x_ref, wq_ref, kt_ref, vt_ref, wo_ref, acc_ref):
        self.x_ref, self.wq_ref = x_ref, wq_ref
        self.kt_ref, self.vt_ref = kt_ref, vt_ref
        self.wo_ref, self.acc_ref = wo_ref, acc_ref
        self.out_ref = self.on_done = None
        self.shared, self.p, self.r, self.p_rest = {}, {}, {}, {}
        self.ot, self.o_rest = {}, {}

    def q_tiles(self):
        q = [None] * 3

        def tile(n, k):
            part = _mm(self.x_ref[:, _tile(k)], self.wq_ref[_tile(k), _tile(n)])
            q[n] = part if k == 0 else q[n] + part
            if (n, k) == (2, D // LANES - 1):
                self._make_lhs([a * Q_SCALE for a in q])

        return [functools.partial(tile, n, k) for n in range(3) for k in range(D // LANES)]

    def _make_lhs(self, q):
        low = _low_lanes(HS)
        x0, x1, x2 = (a[:HS] for a in q)
        y0, y1, y2 = (a[HS:] for a in q)
        y_50 = pltpu.roll(jnp.where(low, y0, y2), HALF, 1)
        d_23 = y1 - _round(x1)
        self.lhs = [_bf16(a) for a in (
            x0 - jnp.where(low, 0.0, _round(y0)),
            jnp.where(low, d_23, y_50),
            jnp.where(low, x1, y0),
            x2 - jnp.where(low, _round(y2), 0.0),
            jnp.where(low, y_50, d_23),
            jnp.where(low, y2, x1),
        )]

    @staticmethod
    def _weights(ref, h, i):
        return jnp.concatenate([ref[j * HALF:(j + 1) * HALF, :] for j in PARTS[h][i]], axis=0)

    def K(self, h, i):
        if i == 0:
            self.shared[h] = _mm(self.lhs[3 * h + 2], self._weights(self.kt_ref, h, 2))
            return
        s = _mm(self.lhs[3 * h + i - 1], self._weights(self.kt_ref, h, i - 1)) + self.shared[h]
        e = jnp.exp2(s - jnp.max(s, axis=1, keepdims=True))
        if i == 2:
            rest = e[LANES - HS:]
            rest = rest * _inverse_row_sum(rest)
            x, y = rest[:REST], rest[REST:]
            self.p_rest[h] = (_bf16(x), _bf16(y), _bf16(x + y))
            e = e[:LANES - HS]
        self.p[h, i] = _bf16(e)
        self.r[h, i] = _inverse_row_sum(self.p[h, i].astype(F32))

    def V(self, h):
        p = jnp.concatenate([self.p[h, 1], self.p[h, 2]], axis=0)
        self.ot[h] = _mm_nt(self.vt_ref[h * DH:(h + 1) * DH, :], p)

    def S(self, h, i):
        self.o_rest[h, i] = _mm_nt(self.p_rest[h][i], self._weights(self.vt_ref, h, i))

    def F(self):
        r0, r1 = (jnp.concatenate([self.r[h, 1], self.r[h, 2]], axis=0) for h in range(2))
        ot0, ot1 = self.ot[0], self.ot[1]
        top = (ot0[:LANES].T, jnp.concatenate([ot0[LANES:], ot1[:HALF]], axis=0).T, ot1[HALF:].T)
        low = _low_lanes(REST)
        a1, a2, a3 = (self.o_rest[0, i] for i in range(3))
        b1, b2, b3 = (self.o_rest[1, i] for i in range(3))
        y_05 = pltpu.roll(jnp.where(low, b2, a2), HALF, 1)
        ox = (a1, jnp.where(low, a3 - a2, b3 - b2), b1)
        oy = (jnp.where(low, y_05, a3 - a1), jnp.where(low, a2, b2), jnp.where(low, b3 - b1, y_05))
        scale = (r0, jnp.where(_low_lanes(LANES), r0, r1), r1)
        self.o = [jnp.concatenate([_bf16(t * r), _bf16(x), _bf16(y)], axis=0)
                  for t, r, x, y in zip(top, scale, ox, oy)]

    def o_tiles(self):
        total = [None]

        def tile(n, k):
            part = _mm(self.o[k], self.wo_ref[_tile(k), _tile(n)])
            total[0] = part if k == 0 else total[0] + part
            if k == 2:
                new = self.acc_ref[:, _tile(n)] + total[0]
                self.acc_ref[:, _tile(n)] = new
                if self.out_ref is not None:
                    self.out_ref[:, _tile(n)] = _bf16(new)
                    if n == D // LANES - 1:
                        self.on_done()

        return [functools.partial(tile, n, k) for n in range(D // LANES) for k in range(3)]


def _run_schedule(schedule, pairs, with_q):
    queue = []

    def issue(count):
        for tile in queue[:count]:
            tile()
        del queue[:count]

    n = len(pairs)
    for t in range(-Q_LEAD, n + O_LAG):
        if with_q and t + Q_LEAD < n:
            queue += pairs[t + Q_LEAD].q_tiles()
        if 0 <= t - O_LAG < n:
            queue += pairs[t - O_LAG].o_tiles()
        both = len(queue) >= 2 * 3 * (D // LANES)
        for op in schedule[1 if both else 0 if t < n // 2 else 2].split():
            if op == "P":
                if len(queue) >= 4:
                    issue(4)
                continue
            i = t if op[0] == "K" else t - 1
            if 0 <= i < n:
                pair = pairs[i]
                {"K": pair.K, "V": pair.V, "S": pair.S, "F": pair.F}[op[0]](*map(int, op[1:]))
        issue(len(queue) // 4 * 4)
    issue(len(queue))


class _Loads:
    def __init__(self, ref):
        self.ref = ref

    def __getitem__(self, i):
        return self.ref[i]


def _kernel(ax, ak, av, awq, awo, bx, bk, bv, bwq, bwo, out,
            x_buf, q_buf, k_buf, v_buf, wq_buf, wo_buf, acc, out_buf,
            x_sem, kv_sem, wq_sem, wo_sem, first_sem, out_sem):
    ks, vs, wqs, wos = (ak, bk), (av, bv), (awq, bwq), (awo, bwo)

    def columns(g):
        return pl.ds(pl.multiple_of(_mod(g, NGQ) * WIDTH, WIDTH), WIDTH)

    def batches(bb):
        return pl.ds(bb * NBAT, NBAT)

    def later_slot(slot, d):
        return jnp.where(slot + d >= NSLOT, slot + d - NSLOT, slot + d)

    def ax_copy(first, count, sem):
        rows = pl.ds(first, count)
        return pltpu.make_async_copy(ax.at[rows], x_buf.at[0, rows], x_sem.at[sem])

    ax_copies = [ax_copy(0, FIRST, 0), ax_copy(FIRST, NBAT - FIRST, 1)]
    ax_copies += [ax_copy(i * NBAT, NBAT, i + 1) for i in range(1, NBB)]
    bx_copy = pltpu.make_async_copy(bx, x_buf.at[1], x_sem.at[NBB + 1])

    def kv_copies(slot, br, i):
        return [pltpu.make_async_copy(src[br].at[batches(_mod(i, NBB)), columns(_div(i, NBB)), :],
                                      buf.at[slot], kv_sem.at[slot])
                for src, buf in ((ks, k_buf), (vs, v_buf))]

    def wq_copies(br, i):
        return [pltpu.make_async_copy(wqs[br].at[:, columns(i)], wq_buf.at[i], wq_sem.at[_mod(i, 2)])]

    def wo_copies(br, i):
        return [pltpu.make_async_copy(wos[br].at[columns(i), :], wo_buf.at[i], wo_sem.at[_mod(i, 2)])]

    def out_copy(br, b):
        cols = pl.ds(pl.multiple_of(br * D, LANES), D)
        return pltpu.make_async_copy(out_buf.at[br, b], out.at[b, :, cols], out_sem)

    def start(copies):
        for copy in copies:
            copy.start()

    def wait(copies):
        for copy in copies:
            copy.wait()

    def on_branch(action, copies, i, per_branch, cond):
        for br in range(2):
            @pl.when(cond & (i >= br * per_branch) & (i < (br + 1) * per_branch))
            def _():
                action(copies(br, i))

    def head_pairs(u, slot):
        g, bb = _div(u, NBB), _mod(u, NBB)
        br = _div(g, NGQ)
        return [_HeadPair(x_buf.at[br, bb * NBAT + j],
                          wq_buf.at[g, :, pl.ds(p * PAIR, PAIR)],
                          k_buf.at[slot, j, pl.ds(p * PAIR, PAIR)],
                          v_buf.at[slot, j, pl.ds(p * PAIR, PAIR)],
                          wo_buf.at[g, pl.ds(p * PAIR, PAIR)],
                          acc.at[br, bb * NBAT + j])
                for j in range(NBAT) for p in range(NPAIR)]

    def project_lead(u, wanted):
        for i, pair in enumerate(head_pairs(u, 0)):
            if wanted(i):
                for tile in pair.q_tiles():
                    tile()
                for j, lhs in enumerate(pair.lhs):
                    q_buf[u, i, j] = lhs

    def clear_acc(u):
        acc[_div(u, NBB), batches(_mod(u, NBB))] = jnp.zeros((NBAT, SQ, D), F32)

    def lead(u, carry):
        @pl.when(_mod(u, NBB) == 0)
        def _():
            wait(wq_copies(0, _div(u, NBB)))

        for i in range(1, NBB):
            pl.when(u == i)(ax_copies[i + 1].wait)

        @pl.when((_mod(u, 2) == 1) & (_div(u, 2) < AHEAD))
        def _():
            start(kv_copies(_div(u, 2), 0, _div(u, 2)))

        clear_acc(u)
        project_lead(u, lambda i: True)
        return carry

    def attend(it, slot, with_q):
        n = STEP if with_q else 1
        u = it * n
        g, bb = _div(u, NBB), _mod(u, NBB)
        br = _div(g, NGQ)
        slots = [slot] + [later_slot(slot, d) for d in range(1, n)]

        @pl.when(bb == 0)
        def _():
            wait(wo_copies(0, g))
            if with_q:
                wait(wq_copies(0, g))

        if with_q:
            pl.when(u == NUNIT // 2)(bx_copy.wait)
        for d in range(n):
            wait(kv_copies(slots[d], 0, u + d))

        on_branch(start, wq_copies, g + 1, NGQ, (bb == 0) & (g + 1 >= LEAD_GROUPS))
        on_branch(start, wo_copies, g + 1, NGQ, bb == 0)
        if with_q:
            pl.when(u == NUNIT // 2 - NBB)(bx_copy.start)
        for d in range(n):
            on_branch(start, functools.partial(kv_copies, later_slot(slot, AHEAD + d)),
                      u + AHEAD + d, NUNIT // 2, True)

        def send(b):
            @pl.when(_mod(g, NGQ) == NGQ - 1)
            def _():
                out_copy(br, b).start()

        pairs = [pair for d in range(n) for pair in head_pairs(u + d, slots[d])]
        for i, pair in enumerate(pairs):
            if not with_q:
                pair.lhs = _Loads(q_buf.at[u, i])
            elif i % NPAIR == NPAIR - 1:
                b = bb * NBAT + i // NPAIR
                pair.out_ref, pair.on_done = out_buf.at[br, b], functools.partial(send, b)
        _run_schedule(SCHEDULE if with_q else SCHEDULE_LEAD, pairs, with_q)
        return later_slot(slot, n)

    first_wq = [pltpu.make_async_copy(awq.at[:, pl.ds(p * PAIR, PAIR)],
                                      wq_buf.at[0, :, pl.ds(p * PAIR, PAIR)], first_sem.at[p])
                for p in range(NPAIR)]

    def in_first_block(i):
        return i % NPAIR == 0 and i // NPAIR < FIRST

    start([first_wq[0], ax_copies[0], first_wq[1], ax_copies[1]])
    clear_acc(0)
    wait([first_wq[0], ax_copies[0]])
    project_lead(0, in_first_block)
    wait([first_wq[1], ax_copies[1]])
    start(ax_copies[2:])
    for g in range(1, LEAD_GROUPS):
        start(wq_copies(0, g))
    start(wo_copies(0, 0))
    project_lead(0, lambda i: not in_first_block(i))

    jax.lax.fori_loop(1, LEAD, lead, 0)
    slot = jax.lax.fori_loop(0, LEAD, functools.partial(attend, with_q=False), 0)
    jax.lax.fori_loop(LEAD // STEP, NUNIT // STEP, functools.partial(attend, with_q=True), slot)
    wait([out_copy(br, b) for br in range(2) for b in range(B)])


@jax.jit
def pallas_concat_heads__gqa_block_cached__mha_block_cached__near_ridge_kernel(
    A_x: jax.Array,
    A_k_cache: jax.Array,
    A_v_cache: jax.Array,
    A_wq: jax.Array,
    A_wo: jax.Array,
    B_x: jax.Array,
    B_k_cache: jax.Array,
    B_v_cache: jax.Array,
    B_wq: jax.Array,
    B_wo: jax.Array,
):
    def transposed(cache):
        assert cache.shape == (B, H, SK, DH), cache.shape
        return jnp.swapaxes(cache, 2, 3).reshape(B, H * DH, SK)

    hbm = pl.BlockSpec(memory_space=pl.ANY)
    dma = pltpu.SemaphoreType.DMA
    return pl.pallas_call(
        _kernel,
        in_specs=[hbm] * 10,
        out_specs=hbm,
        out_shape=jax.ShapeDtypeStruct((B, SQ, 2 * D), BF16),
        scratch_shapes=[
            pltpu.VMEM((2, B, SQ, D), BF16),
            pltpu.VMEM((LEAD, NBAT * NPAIR, 6, HS, LANES), BF16),
            pltpu.VMEM((NSLOT, NBAT, WIDTH, SK), BF16),
            pltpu.VMEM((NSLOT, NBAT, WIDTH, SK), BF16),
            pltpu.VMEM((NGROUP, D, WIDTH), BF16),
            pltpu.VMEM((NGROUP, WIDTH, D), BF16),
            pltpu.VMEM((2, B, SQ, D), F32),
            pltpu.VMEM((2, B, SQ, D), BF16),
            dma((NBB + 2,)), dma((NSLOT,)), dma((2,)), dma((2,)), dma((NPAIR,)), dma(()),
        ],
        compiler_params=pltpu.CompilerParams(
            vmem_limit_bytes=124 * 1024 * 1024, disable_bounds_checks=True),
        name="attn_kernel",
    )(A_x, transposed(A_k_cache), transposed(A_v_cache), A_wq, A_wo,
      B_x, transposed(B_k_cache), transposed(B_v_cache), B_wq, B_wo)
```

```python
import functools

import jax
import jax.experimental.pallas as pl
import jax.experimental.pallas.tpu as pltpu
import jax.numpy as jnp
import numpy as np

B, SQ, D = 16, 160, 640
H, SK, DH = 32, 512, 192

LANES = 128
HALF = LANES // 2
PAIR = 2 * DH
HS = SQ // 2
REST = (SQ - LANES) // 2
Q_SCALE = float(DH ** -0.5 * np.log2(np.e))

NBAT, NPAIR = 4, 2
STEP = 2
LEAD = 8
NSLOT = 6
FIRST = 2

NBB = B // NBAT
NGQ = H // (2 * NPAIR)
WIDTH = NPAIR * PAIR
NGROUP = 2 * NGQ
NUNIT = NGROUP * NBB
AHEAD = NSLOT - STEP
LEAD_GROUPS = LEAD // NBB
assert NPAIR == 2 and LEAD == 2 * NBB and NBB % STEP == 0
assert 2 * AHEAD <= LEAD <= NUNIT // 2 - NBB

PARTS = (((0, 1), (2, 0), (2, 1)), ((4, 5), (5, 3), (4, 3)))

SCHEDULE = (
    "K00 K10 S01 K02 K12 K01 S10 K11 V0 S02 P P S00 V1 S12 S11 F",
    "P P P K00 S01 K02 K10 P K12 K01 S10 V0 S02 P P S00 V1 S11 S12 P F P K11",
    "K00 S00 K10 K12 S10 V0 K02 S02 P P K01 K11 S12 V1 S01 S11 F P",
)
SCHEDULE_LEAD = ("K00 K02 S00 K10 K12 S10 V0 S02 P P K01 K11 S12 V1 S01 S11 F P",) * 3
Q_LEAD, O_LAG = 2, 3

F32, BF16 = jnp.float32, jnp.bfloat16


def _mm(a, b):
    return jnp.dot(a, b, preferred_element_type=F32)


def _mm_nt(a, b):
    return jax.lax.dot_general(a, b, (((1,), (1,)), ((), ())), preferred_element_type=F32)


def _bf16(a):
    return a.astype(BF16)


def _round(a):
    return a.astype(BF16).astype(F32)


def _tile(i):
    return slice(i * LANES, (i + 1) * LANES)


def _low_lanes(rows):
    return jax.lax.broadcasted_iota(jnp.int32, (rows, LANES), 1) < HALF


def _inverse_row_sum(p):
    total = jnp.sum(p, axis=1, keepdims=True)
    r = pl.reciprocal(total, approx=True)
    return r * (2.0 - total * r)


def _div(a, n):
    return a >> (n.bit_length() - 1)


def _mod(a, n):
    return a & (n - 1)


class _HeadPair:
    def __init__(self, x_ref, wq_ref, kt_ref, vt_ref, wo_ref, acc_ref):
        self.x_ref, self.wq_ref = x_ref, wq_ref
        self.kt_ref, self.vt_ref = kt_ref, vt_ref
        self.wo_ref, self.acc_ref = wo_ref, acc_ref
        self.out_ref = self.on_done = None
        self.shared, self.p, self.r, self.p_rest = {}, {}, {}, {}
        self.ot, self.o_rest = {}, {}

    def q_tiles(self, order=(0, 1, 2)):
        q = [None] * 3

        def tile(n, k):
            part = _mm(self.x_ref[:, _tile(k)], self.wq_ref[_tile(k), _tile(n)])
            q[n] = part if k == 0 else q[n] + part
            if (n, k) == (order[-1], D // LANES - 1):
                self._make_lhs([a * Q_SCALE for a in q])

        return [functools.partial(tile, n, k) for n in order for k in range(D // LANES)]

    def _make_lhs(self, q):
        low = _low_lanes(HS)
        x0, x1, x2 = (a[:HS] for a in q)
        y0, y1, y2 = (a[HS:] for a in q)
        y_50 = pltpu.roll(jnp.where(low, y0, y2), HALF, 1)
        d_23 = y1 - _round(x1)
        self.lhs = [_bf16(a) for a in (
            x0 - jnp.where(low, 0.0, _round(y0)),
            jnp.where(low, d_23, y_50),
            jnp.where(low, x1, y0),
            x2 - jnp.where(low, _round(y2), 0.0),
            jnp.where(low, y_50, d_23),
            jnp.where(low, y2, x1),
        )]

    @staticmethod
    def _weights(ref, h, i):
        return jnp.concatenate([ref[j * HALF:(j + 1) * HALF, :] for j in PARTS[h][i]], axis=0)

    def K(self, h, i):
        if i == 0:
            self.shared[h] = _mm(self.lhs[3 * h + 2], self._weights(self.kt_ref, h, 2))
            return
        s = _mm(self.lhs[3 * h + i - 1], self._weights(self.kt_ref, h, i - 1)) + self.shared[h]
        e = jnp.exp2(s - jnp.max(s, axis=1, keepdims=True))
        if i == 2:
            rest = e[LANES - HS:]
            rest = rest * _inverse_row_sum(rest)
            x, y = rest[:REST], rest[REST:]
            self.p_rest[h] = (_bf16(x), _bf16(y), _bf16(x + y))
            e = e[:LANES - HS]
        self.p[h, i] = _bf16(e)
        self.r[h, i] = _inverse_row_sum(self.p[h, i].astype(F32))

    def V(self, h):
        p = jnp.concatenate([self.p[h, 1], self.p[h, 2]], axis=0)
        self.ot[h] = _mm_nt(self.vt_ref[h * DH:(h + 1) * DH, :], p)

    def S(self, h, i):
        self.o_rest[h, i] = _mm_nt(self.p_rest[h][i], self._weights(self.vt_ref, h, i))

    def F(self):
        r0, r1 = (jnp.concatenate([self.r[h, 1], self.r[h, 2]], axis=0) for h in range(2))
        ot0, ot1 = self.ot[0], self.ot[1]
        top = (ot0[:LANES].T, jnp.concatenate([ot0[LANES:], ot1[:HALF]], axis=0).T, ot1[HALF:].T)
        low = _low_lanes(REST)
        a1, a2, a3 = (self.o_rest[0, i] for i in range(3))
        b1, b2, b3 = (self.o_rest[1, i] for i in range(3))
        y_05 = pltpu.roll(jnp.where(low, b2, a2), HALF, 1)
        ox = (a1, jnp.where(low, a3 - a2, b3 - b2), b1)
        oy = (jnp.where(low, y_05, a3 - a1), jnp.where(low, a2, b2), jnp.where(low, b3 - b1, y_05))
        scale = (r0, jnp.where(_low_lanes(LANES), r0, r1), r1)
        self.o = [jnp.concatenate([_bf16(t * r), _bf16(x), _bf16(y)], axis=0)
                  for t, r, x, y in zip(top, scale, ox, oy)]

    def o_tiles(self):
        total = [None]

        def tile(n, k):
            part = _mm(self.o[k], self.wo_ref[_tile(k), _tile(n)])
            total[0] = part if k == 0 else total[0] + part
            if k == 2:
                new = self.acc_ref[:, _tile(n)] + total[0]
                self.acc_ref[:, _tile(n)] = new
                if self.out_ref is not None:
                    self.out_ref[:, _tile(n)] = _bf16(new)
                    if n == D // LANES - 1:
                        self.on_done()

        return [functools.partial(tile, n, k) for n in range(D // LANES) for k in range(3)]


def _run_schedule(schedule, pairs, with_q):
    queue = []

    def issue(count):
        for tile in queue[:count]:
            tile()
        del queue[:count]

    n = len(pairs)
    for t in range(-Q_LEAD, n + O_LAG):
        if with_q and t + Q_LEAD < n:
            queue += pairs[t + Q_LEAD].q_tiles()
        if 0 <= t - O_LAG < n:
            queue += pairs[t - O_LAG].o_tiles()
        both = len(queue) >= 2 * 3 * (D // LANES)
        for op in schedule[1 if both else 0 if t < n // 2 else 2].split():
            if op == "P":
                if len(queue) >= 4:
                    issue(4)
                continue
            i = t if op[0] == "K" else t - 1
            if 0 <= i < n:
                pair = pairs[i]
                {"K": pair.K, "V": pair.V, "S": pair.S, "F": pair.F}[op[0]](*map(int, op[1:]))
        issue(len(queue) // 4 * 4)
    issue(len(queue))


class _Loads:
    def __init__(self, ref):
        self.ref = ref

    def __getitem__(self, i):
        return self.ref[i]


def _kernel(ax, ak, av, awq, awo, bx, bk, bv, bwq, bwo, out,
            x_buf, q_buf, k_buf, v_buf, wq_buf, wo_buf, acc, out_buf,
            x_sem, kv_sem, wq_sem, wo_sem, first_sem, out_sem):
    ks, vs, wqs, wos = (ak, bk), (av, bv), (awq, bwq), (awo, bwo)

    def columns(g):
        return pl.ds(pl.multiple_of(_mod(g, NGQ) * WIDTH, WIDTH), WIDTH)

    def batches(bb):
        return pl.ds(bb * NBAT, NBAT)

    def later_slot(slot, d):
        return jnp.where(slot + d >= NSLOT, slot + d - NSLOT, slot + d)

    def ax_copy(first, count, sem):
        rows = pl.ds(first, count)
        return pltpu.make_async_copy(ax.at[rows], x_buf.at[0, rows], x_sem.at[sem])

    ax_copies = [ax_copy(0, FIRST, 0), ax_copy(FIRST, NBAT - FIRST, 1)]
    ax_copies += [ax_copy(i * NBAT, NBAT, i + 1) for i in range(1, NBB)]
    bx_copy = pltpu.make_async_copy(bx, x_buf.at[1], x_sem.at[NBB + 1])

    def kv_copies(slot, br, i):
        return [pltpu.make_async_copy(src[br].at[batches(_mod(i, NBB)), columns(_div(i, NBB)), :],
                                      buf.at[slot], kv_sem.at[slot])
                for src, buf in ((ks, k_buf), (vs, v_buf))]

    def wq_copies(br, i):
        return [pltpu.make_async_copy(wqs[br].at[:, columns(i)], wq_buf.at[i], wq_sem.at[_mod(i, 2)])]

    def wo_copies(br, i):
        return [pltpu.make_async_copy(wos[br].at[columns(i), :], wo_buf.at[i], wo_sem.at[_mod(i, 2)])]

    def out_copy(br, b):
        cols = pl.ds(pl.multiple_of(br * D, LANES), D)
        return pltpu.make_async_copy(out_buf.at[br, b], out.at[b, :, cols], out_sem)

    def start(copies):
        for copy in copies:
            copy.start()

    def wait(copies):
        for copy in copies:
            copy.wait()

    def on_branch(action, copies, i, per_branch, cond):
        for br in range(2):
            @pl.when(cond & (i >= br * per_branch) & (i < (br + 1) * per_branch))
            def _():
                action(copies(br, i))

    def head_pairs(u, slot):
        g, bb = _div(u, NBB), _mod(u, NBB)
        br = _div(g, NGQ)
        return [_HeadPair(x_buf.at[br, bb * NBAT + j],
                          wq_buf.at[g, :, pl.ds(p * PAIR, PAIR)],
                          k_buf.at[slot, j, pl.ds(p * PAIR, PAIR)],
                          v_buf.at[slot, j, pl.ds(p * PAIR, PAIR)],
                          wo_buf.at[g, pl.ds(p * PAIR, PAIR)],
                          acc.at[br, bb * NBAT + j])
                for j in range(NBAT) for p in range(NPAIR)]

    def project_lead(u, wanted):
        for i, pair in enumerate(head_pairs(u, 0)):
            if wanted(i):
                for tile in pair.q_tiles(order=(0, 2, 1)):
                    tile()
                for j, lhs in enumerate(pair.lhs):
                    q_buf[u, i, j] = lhs

    def clear_acc(u):
        acc[_div(u, NBB), batches(_mod(u, NBB))] = jnp.zeros((NBAT, SQ, D), F32)

    def lead(u, carry):
        @pl.when(_mod(u, NBB) == 0)
        def _():
            wait(wq_copies(0, _div(u, NBB)))

        for i in range(1, NBB):
            pl.when(u == i)(ax_copies[i + 1].wait)

        @pl.when((_mod(u, 2) == 1) & (_div(u, 2) < AHEAD))
        def _():
            start(kv_copies(_div(u, 2), 0, _div(u, 2)))

        clear_acc(u)
        project_lead(u, lambda i: True)
        return carry

    def attend(it, slot, with_q):
        n = STEP if with_q else 1
        u = it * n
        g, bb = _div(u, NBB), _mod(u, NBB)
        br = _div(g, NGQ)
        slots = [slot] + [later_slot(slot, d) for d in range(1, n)]

        @pl.when(bb == 0)
        def _():
            wait(wo_copies(0, g))
            if with_q:
                wait(wq_copies(0, g))

        if with_q:
            pl.when(u == NUNIT // 2)(bx_copy.wait)
        for d in range(n):
            wait(kv_copies(slots[d], 0, u + d))

        on_branch(start, wq_copies, g + 1, NGQ, (bb == 0) & (g + 1 >= LEAD_GROUPS))
        on_branch(start, wo_copies, g + 1, NGQ, bb == 0)
        if with_q:
            pl.when(u == NUNIT // 2 - NBB)(bx_copy.start)
        for d in range(n):
            on_branch(start, functools.partial(kv_copies, later_slot(slot, AHEAD + d)),
                      u + AHEAD + d, NUNIT // 2, True)

        def send(b):
            @pl.when(_mod(g, NGQ) == NGQ - 1)
            def _():
                out_copy(br, b).start()

        pairs = [pair for d in range(n) for pair in head_pairs(u + d, slots[d])]
        for i, pair in enumerate(pairs):
            if not with_q:
                pair.lhs = _Loads(q_buf.at[u, i])
            elif i % NPAIR == NPAIR - 1:
                b = bb * NBAT + i // NPAIR
                pair.out_ref, pair.on_done = out_buf.at[br, b], functools.partial(send, b)
        _run_schedule(SCHEDULE if with_q else SCHEDULE_LEAD, pairs, with_q)
        return later_slot(slot, n)

    first_wq = [pltpu.make_async_copy(awq.at[:, pl.ds(p * PAIR, PAIR)],
                                      wq_buf.at[0, :, pl.ds(p * PAIR, PAIR)], first_sem.at[p])
                for p in range(NPAIR)]

    def in_first_block(i):
        return i % NPAIR == 0 and i // NPAIR < FIRST

    start([first_wq[0], ax_copies[0], first_wq[1], ax_copies[1]])
    clear_acc(0)
    wait([first_wq[0], ax_copies[0]])
    project_lead(0, in_first_block)
    wait([first_wq[1], ax_copies[1]])
    start(ax_copies[2:])
    for g in range(1, LEAD_GROUPS):
        start(wq_copies(0, g))
    start(wo_copies(0, 0))
    project_lead(0, lambda i: not in_first_block(i))

    jax.lax.fori_loop(1, LEAD, lead, 0)
    slot = jax.lax.fori_loop(0, LEAD, functools.partial(attend, with_q=False), 0)
    jax.lax.fori_loop(LEAD // STEP, NUNIT // STEP, functools.partial(attend, with_q=True), slot)
    wait([out_copy(br, b) for br in range(2) for b in range(B)])


@jax.jit
def pallas_concat_heads__gqa_block_cached__mha_block_cached__near_ridge_kernel(
    A_x: jax.Array,
    A_k_cache: jax.Array,
    A_v_cache: jax.Array,
    A_wq: jax.Array,
    A_wo: jax.Array,
    B_x: jax.Array,
    B_k_cache: jax.Array,
    B_v_cache: jax.Array,
    B_wq: jax.Array,
    B_wo: jax.Array,
):
    def transposed(cache):
        assert cache.shape == (B, H, SK, DH), cache.shape
        return jnp.swapaxes(cache, 2, 3).reshape(B, H * DH, SK)

    hbm = pl.BlockSpec(memory_space=pl.ANY)
    dma = pltpu.SemaphoreType.DMA
    return pl.pallas_call(
        _kernel,
        in_specs=[hbm] * 10,
        out_specs=hbm,
        out_shape=jax.ShapeDtypeStruct((B, SQ, 2 * D), BF16),
        scratch_shapes=[
            pltpu.VMEM((2, B, SQ, D), BF16),
            pltpu.VMEM((LEAD, NBAT * NPAIR, 6, HS, LANES), BF16),
            pltpu.VMEM((NSLOT, NBAT, WIDTH, SK), BF16),
            pltpu.VMEM((NSLOT, NBAT, WIDTH, SK), BF16),
            pltpu.VMEM((NGROUP, D, WIDTH), BF16),
            pltpu.VMEM((NGROUP, WIDTH, D), BF16),
            pltpu.VMEM((2, B, SQ, D), F32),
            pltpu.VMEM((2, B, SQ, D), BF16),
            dma((NBB + 2,)), dma((NSLOT,)), dma((2,)), dma((2,)), dma((NPAIR,)), dma(()),
        ],
        compiler_params=pltpu.CompilerParams(
            vmem_limit_bytes=124 * 1024 * 1024, disable_bounds_checks=True),
        name="attn_kernel",
    )(A_x, transposed(A_k_cache), transposed(A_v_cache), A_wq, A_wo,
      B_x, transposed(B_k_cache), transposed(B_v_cache), B_wq, B_wo)
```

```python
import functools

import jax
import jax.experimental.pallas as pl
import jax.experimental.pallas.tpu as pltpu
import jax.numpy as jnp
import numpy as np

B, SQ, D = 16, 160, 640
H, SK, DH = 32, 512, 192

LANES = 128
HALF = LANES // 2
PAIR = 2 * DH
HS = SQ // 2
REST = (SQ - LANES) // 2
Q_SCALE = float(DH ** -0.5 * np.log2(np.e))

NBAT, NPAIR = 4, 2
STEP = 2
LEAD = 8
NSLOT = 6
FIRST = 2

NBB = B // NBAT
NGQ = H // (2 * NPAIR)
WIDTH = NPAIR * PAIR
NGROUP = 2 * NGQ
NUNIT = NGROUP * NBB
AHEAD = NSLOT - STEP
LEAD_GROUPS = LEAD // NBB
assert NPAIR == 2 and LEAD == 2 * NBB and NBB % STEP == 0
assert 2 * AHEAD <= LEAD <= NUNIT // 2 - NBB

PARTS = (((0, 1), (2, 0), (2, 1)), ((4, 5), (5, 3), (4, 3)))

SCHEDULE = (
    "K00 K10 S01 K02 K12 K01 S10 K11 V0 S02 P P S00 V1 S12 S11 F",
    "P P P K00 S01 K02 K10 P K12 K01 S10 V0 S02 P P S00 V1 S12 S11 P F P K11",
    "K00 K10 S00 K11 K12 S10 V0 K02 S02 P P K01 S12 V1 S01 S11 F P",
)
SCHEDULE_LEAD = ("K00 K02 S00 K10 K12 S10 V0 S02 P P K01 K11 S12 V1 S01 S11 F P",) * 3
Q_LEAD, O_LAG = 2, 3

F32, BF16 = jnp.float32, jnp.bfloat16
_reciprocal = pltpu.reciprocal if hasattr(pltpu, "reciprocal") else pl.reciprocal


def _mm(a, b):
    return jnp.dot(a, b, preferred_element_type=F32)


def _mm_nt(a, b):
    return jax.lax.dot_general(a, b, (((1,), (1,)), ((), ())), preferred_element_type=F32)


def _bf16(a):
    return a.astype(BF16)


def _round(a):
    return a.astype(BF16).astype(F32)


def _tile(i):
    return slice(i * LANES, (i + 1) * LANES)


def _low_lanes(rows):
    return jax.lax.broadcasted_iota(jnp.int32, (rows, LANES), 1) < HALF


def _inverse_row_sum(p):
    total = jnp.sum(p, axis=1, keepdims=True)
    r = _reciprocal(total, approx=True)
    return r * (2.0 - total * r)


def _div(a, n):
    return a >> (n.bit_length() - 1)


def _mod(a, n):
    return a & (n - 1)


class _HeadPair:
    def __init__(self, x_ref, wq_ref, kt_ref, vt_ref, wo_ref, acc_ref):
        self.x_ref, self.wq_ref = x_ref, wq_ref
        self.kt_ref, self.vt_ref = kt_ref, vt_ref
        self.wo_ref, self.acc_ref = wo_ref, acc_ref
        self.out_ref = self.on_done = None
        self.shared, self.p, self.r, self.p_rest = {}, {}, {}, {}
        self.ot, self.o_rest = {}, {}

    def q_tiles(self, order=(0, 1, 2)):
        q = [None] * 3

        def tile(n, k):
            part = _mm(self.x_ref[:, _tile(k)], self.wq_ref[_tile(k), _tile(n)])
            q[n] = part if k == 0 else q[n] + part
            if (n, k) == (order[-1], D // LANES - 1):
                self._make_lhs([a * Q_SCALE for a in q])

        return [functools.partial(tile, n, k) for n in order for k in range(D // LANES)]

    def _make_lhs(self, q):
        low = _low_lanes(HS)
        x0, x1, x2 = (a[:HS] for a in q)
        y0, y1, y2 = (a[HS:] for a in q)
        y_50 = pltpu.roll(jnp.where(low, y0, y2), HALF, 1)
        d_23 = y1 - _round(x1)
        self.lhs = [_bf16(a) for a in (
            x0 - jnp.where(low, 0.0, _round(y0)),
            jnp.where(low, d_23, y_50),
            jnp.where(low, x1, y0),
            x2 - jnp.where(low, _round(y2), 0.0),
            jnp.where(low, y_50, d_23),
            jnp.where(low, y2, x1),
        )]

    @staticmethod
    def _weights(ref, h, i):
        return jnp.concatenate([ref[j * HALF:(j + 1) * HALF, :] for j in PARTS[h][i]], axis=0)

    def K(self, h, i):
        if i == 0:
            self.shared[h] = _mm(self.lhs[3 * h + 2], self._weights(self.kt_ref, h, 2))
            return
        s = _mm(self.lhs[3 * h + i - 1], self._weights(self.kt_ref, h, i - 1)) + self.shared[h]
        e = jnp.exp2(s - jnp.max(s, axis=1, keepdims=True))
        if i == 2:
            rest = e[LANES - HS:]
            rest = rest * _inverse_row_sum(rest)
            x, y = rest[:REST], rest[REST:]
            self.p_rest[h] = (_bf16(x), _bf16(y), _bf16(x + y))
            e = e[:LANES - HS]
        self.p[h, i] = _bf16(e)
        self.r[h, i] = _inverse_row_sum(self.p[h, i].astype(F32))

    def V(self, h):
        p = jnp.concatenate([self.p[h, 1], self.p[h, 2]], axis=0)
        self.ot[h] = _mm_nt(self.vt_ref[h * DH:(h + 1) * DH, :], p)

    def S(self, h, i):
        self.o_rest[h, i] = _mm_nt(self.p_rest[h][i], self._weights(self.vt_ref, h, i))

    def F(self):
        r0, r1 = (jnp.concatenate([self.r[h, 1], self.r[h, 2]], axis=0) for h in range(2))
        ot0, ot1 = self.ot[0], self.ot[1]
        top = (ot0[:LANES].T, jnp.concatenate([ot0[LANES:], ot1[:HALF]], axis=0).T, ot1[HALF:].T)
        low = _low_lanes(REST)
        a1, a2, a3 = (self.o_rest[0, i] for i in range(3))
        b1, b2, b3 = (self.o_rest[1, i] for i in range(3))
        y_05 = pltpu.roll(jnp.where(low, b2, a2), HALF, 1)
        ox = (a1, jnp.where(low, a3 - a2, b3 - b2), b1)
        oy = (jnp.where(low, y_05, a3 - a1), jnp.where(low, a2, b2), jnp.where(low, b3 - b1, y_05))
        scale = (r0, jnp.where(_low_lanes(LANES), r0, r1), r1)
        self.o = [jnp.concatenate([_bf16(t * r), _bf16(x), _bf16(y)], axis=0)
                  for t, r, x, y in zip(top, scale, ox, oy)]

    def o_tiles(self):
        total = [None]

        def tile(n, k):
            part = _mm(self.o[k], self.wo_ref[_tile(k), _tile(n)])
            total[0] = part if k == 0 else total[0] + part
            if k == 2:
                new = self.acc_ref[:, _tile(n)] + total[0]
                self.acc_ref[:, _tile(n)] = new
                if self.out_ref is not None:
                    self.out_ref[:, _tile(n)] = _bf16(new)
                    if n == D // LANES - 1:
                        self.on_done()

        return [functools.partial(tile, n, k) for n in range(D // LANES) for k in range(3)]


def _run_schedule(schedule, pairs, with_q):
    queue = []

    def issue(count):
        for tile in queue[:count]:
            tile()
        del queue[:count]

    n = len(pairs)
    for t in range(-Q_LEAD, n + O_LAG):
        if with_q and t + Q_LEAD < n:
            queue += pairs[t + Q_LEAD].q_tiles()
        if 0 <= t - O_LAG < n:
            queue += pairs[t - O_LAG].o_tiles()
        both = len(queue) >= 2 * 3 * (D // LANES)
        for op in schedule[1 if both else 0 if t < n // 2 else 2].split():
            if op == "P":
                if len(queue) >= 4:
                    issue(4)
                continue
            i = t if op[0] == "K" else t - 1
            if 0 <= i < n:
                pair = pairs[i]
                {"K": pair.K, "V": pair.V, "S": pair.S, "F": pair.F}[op[0]](*map(int, op[1:]))
        issue(len(queue) // 4 * 4)
    issue(len(queue))


class _Loads:
    def __init__(self, ref):
        self.ref = ref

    def __getitem__(self, i):
        return self.ref[i]


def _kernel(ax, ak, av, awq, awo, bx, bk, bv, bwq, bwo, out,
            x_buf, q_buf, k_buf, v_buf, wq_buf, wo_buf, acc, out_buf,
            x_sem, kv_sem, wq_sem, wo_sem, first_sem, out_sem):
    ks, vs, wqs, wos = (ak, bk), (av, bv), (awq, bwq), (awo, bwo)

    def columns(g):
        return pl.ds(pl.multiple_of(_mod(g, NGQ) * WIDTH, WIDTH), WIDTH)

    def batches(bb):
        return pl.ds(bb * NBAT, NBAT)

    def later_slot(slot, d):
        return jnp.where(slot + d >= NSLOT, slot + d - NSLOT, slot + d)

    def ax_copy(first, count, sem):
        rows = pl.ds(first, count)
        return pltpu.make_async_copy(ax.at[rows], x_buf.at[0, rows], x_sem.at[sem])

    ax_copies = [ax_copy(0, FIRST, 0), ax_copy(FIRST, NBAT - FIRST, 1)]
    ax_copies += [ax_copy(i * NBAT, NBAT, i + 1) for i in range(1, NBB)]
    bx_copy = pltpu.make_async_copy(bx, x_buf.at[1], x_sem.at[NBB + 1])

    def kv_copies(slot, br, i):
        return [pltpu.make_async_copy(src[br].at[batches(_mod(i, NBB)), columns(_div(i, NBB)), :],
                                      buf.at[slot], kv_sem.at[slot])
                for src, buf in ((ks, k_buf), (vs, v_buf))]

    def wq_copies(br, i):
        return [pltpu.make_async_copy(wqs[br].at[:, columns(i)], wq_buf.at[i], wq_sem.at[_mod(i, 2)])]

    def wo_copies(br, i):
        return [pltpu.make_async_copy(wos[br].at[columns(i), :], wo_buf.at[i], wo_sem.at[_mod(i, 2)])]

    def out_copy(br, b):
        cols = pl.ds(pl.multiple_of(br * D, LANES), D)
        return pltpu.make_async_copy(out_buf.at[br, b], out.at[b, :, cols], out_sem)

    def start(copies):
        for copy in copies:
            copy.start()

    def wait(copies):
        for copy in copies:
            copy.wait()

    def on_branch(action, copies, i, per_branch, cond):
        for br in range(2):
            @pl.when(cond & (i >= br * per_branch) & (i < (br + 1) * per_branch))
            def _():
                action(copies(br, i))

    def head_pairs(u, slot):
        g, bb = _div(u, NBB), _mod(u, NBB)
        br = _div(g, NGQ)
        return [_HeadPair(x_buf.at[br, bb * NBAT + j],
                          wq_buf.at[g, :, pl.ds(p * PAIR, PAIR)],
                          k_buf.at[slot, j, pl.ds(p * PAIR, PAIR)],
                          v_buf.at[slot, j, pl.ds(p * PAIR, PAIR)],
                          wo_buf.at[g, pl.ds(p * PAIR, PAIR)],
                          acc.at[br, bb * NBAT + j])
                for j in range(NBAT) for p in range(NPAIR)]

    def project_lead(u, wanted):
        for i, pair in enumerate(head_pairs(u, 0)):
            if wanted(i):
                for tile in pair.q_tiles(order=(0, 2, 1)):
                    tile()
                for j, lhs in enumerate(pair.lhs):
                    q_buf[u, i, j] = lhs

    def clear_acc(u):
        acc[_div(u, NBB), batches(_mod(u, NBB))] = jnp.zeros((NBAT, SQ, D), F32)

    def lead(u, carry):
        @pl.when(_mod(u, NBB) == 0)
        def _():
            wait(wq_copies(0, _div(u, NBB)))

        for i in range(1, NBB):
            pl.when(u == i)(ax_copies[i + 1].wait)

        @pl.when((_mod(u, 2) == 1) & (_div(u, 2) < AHEAD))
        def _():
            start(kv_copies(_div(u, 2), 0, _div(u, 2)))

        clear_acc(u)
        project_lead(u, lambda i: True)
        return carry

    def attend(it, slot, with_q):
        n = STEP if with_q else 1
        u = it * n
        g, bb = _div(u, NBB), _mod(u, NBB)
        br = _div(g, NGQ)
        slots = [slot] + [later_slot(slot, d) for d in range(1, n)]

        @pl.when(bb == 0)
        def _():
            wait(wo_copies(0, g))
            if with_q:
                wait(wq_copies(0, g))

        if with_q:
            pl.when(u == NUNIT // 2)(bx_copy.wait)
        for d in range(n):
            wait(kv_copies(slots[d], 0, u + d))

        on_branch(start, wq_copies, g + 1, NGQ, (bb == 0) & (g + 1 >= LEAD_GROUPS))
        on_branch(start, wo_copies, g + 1, NGQ, bb == 0)
        if with_q:
            pl.when(u == NUNIT // 2 - NBB)(bx_copy.start)
        for d in range(n):
            on_branch(start, functools.partial(kv_copies, later_slot(slot, AHEAD + d)),
                      u + AHEAD + d, NUNIT // 2, True)

        def send(b):
            @pl.when(_mod(g, NGQ) == NGQ - 1)
            def _():
                out_copy(br, b).start()

        pairs = [pair for d in range(n) for pair in head_pairs(u + d, slots[d])]
        for i, pair in enumerate(pairs):
            if not with_q:
                pair.lhs = _Loads(q_buf.at[u, i])
            elif i % NPAIR == NPAIR - 1:
                b = bb * NBAT + i // NPAIR
                pair.out_ref, pair.on_done = out_buf.at[br, b], functools.partial(send, b)
        _run_schedule(SCHEDULE if with_q else SCHEDULE_LEAD, pairs, with_q)
        return later_slot(slot, n)

    first_wq = [pltpu.make_async_copy(awq.at[:, pl.ds(p * PAIR, PAIR)],
                                      wq_buf.at[0, :, pl.ds(p * PAIR, PAIR)], first_sem.at[p])
                for p in range(NPAIR)]

    def in_first_block(i):
        return i % NPAIR == 0 and i // NPAIR < FIRST

    start([first_wq[0], ax_copies[0], first_wq[1], ax_copies[1]])
    clear_acc(0)
    wait([first_wq[0], ax_copies[0]])
    project_lead(0, in_first_block)
    wait([first_wq[1], ax_copies[1]])
    start(ax_copies[2:])
    for g in range(1, LEAD_GROUPS):
        start(wq_copies(0, g))
    start(wo_copies(0, 0))
    project_lead(0, lambda i: not in_first_block(i))

    jax.lax.fori_loop(1, LEAD, lead, 0)
    slot = jax.lax.fori_loop(0, LEAD, functools.partial(attend, with_q=False), 0)
    jax.lax.fori_loop(LEAD // STEP, NUNIT // STEP, functools.partial(attend, with_q=True), slot)
    wait([out_copy(br, b) for br in range(2) for b in range(B)])


@jax.jit
def pallas_concat_heads__gqa_block_cached__mha_block_cached__near_ridge_kernel(
    A_x: jax.Array,
    A_k_cache: jax.Array,
    A_v_cache: jax.Array,
    A_wq: jax.Array,
    A_wo: jax.Array,
    B_x: jax.Array,
    B_k_cache: jax.Array,
    B_v_cache: jax.Array,
    B_wq: jax.Array,
    B_wo: jax.Array,
):
    def transposed(cache):
        assert cache.shape == (B, H, SK, DH), cache.shape
        return jnp.swapaxes(cache, 2, 3).reshape(B, H * DH, SK)

    hbm = pl.BlockSpec(memory_space=pl.ANY)
    dma = pltpu.SemaphoreType.DMA
    return pl.pallas_call(
        _kernel,
        in_specs=[hbm] * 10,
        out_specs=hbm,
        out_shape=jax.ShapeDtypeStruct((B, SQ, 2 * D), BF16),
        scratch_shapes=[
            pltpu.VMEM((2, B, SQ, D), BF16),
            pltpu.VMEM((LEAD, NBAT * NPAIR, 6, HS, LANES), BF16),
            pltpu.VMEM((NSLOT, NBAT, WIDTH, SK), BF16),
            pltpu.VMEM((NSLOT, NBAT, WIDTH, SK), BF16),
            pltpu.VMEM((NGROUP, D, WIDTH), BF16),
            pltpu.VMEM((NGROUP, WIDTH, D), BF16),
            pltpu.VMEM((2, B, SQ, D), F32),
            pltpu.VMEM((2, B, SQ, D), BF16),
            dma((NBB + 2,)), dma((NSLOT,)), dma((2,)), dma((2,)), dma((NPAIR,)), dma(()),
        ],
        compiler_params=pltpu.CompilerParams(
            vmem_limit_bytes=124 * 1024 * 1024, disable_bounds_checks=True),
        name="attn_kernel",
    )(A_x, transposed(A_k_cache), transposed(A_v_cache), A_wq, A_wo,
      B_x, transposed(B_k_cache), transposed(B_v_cache), B_wq, B_wo)
```
